```python
import jax
import jax.numpy as jnp

def _softmax(x, axis=-1):
    return jax.nn.softmax(x, axis=axis)
def _gelu(x):
    return jax.nn.gelu(x, approximate=True)
def _silu(x):
    return jax.nn.silu(x)
def _sigmoid(x):
    return jax.nn.sigmoid(x)
def _layernorm(x, axis=-1, eps=1e-5):
    m = jnp.mean(x, axis=axis, keepdims=True)
    v = jnp.var(x, axis=axis, keepdims=True)
    return (x - m) / jnp.sqrt(v + eps)
def _scatter_add(tgt, idx, src, axis=0):
    return tgt.at[idx].add(src)
def _segment_sum(src, seg, n):
    return jax.ops.segment_sum(src, seg, n)
class _Rng:
    def __init__(self, key):
        self._k = key
    def _next(self):
        self._k, sub = jax.random.split(self._k)
        return sub
    def normal(self, shape):
        return jax.random.normal(self._next(), shape, dtype=jnp.bfloat16)
    def randint(self, lo, hi, shape):
        return jax.random.randint(self._next(), shape, lo, hi, dtype=jnp.int32)
    def uniform(self, shape, lo=0.0, hi=1.0):
        return jax.random.uniform(self._next(), shape, jnp.bfloat16, lo, hi)
    def permutation(self, n):
        return jax.random.permutation(self._next(), n)


kernel_name = 'gated_mix__compressed_kv_cla__moe_arch_mod__prompt'

def setup_inputs():
    _rng = _Rng(jax.random.key(int.from_bytes(__import__("os").urandom(4), "little")))
    _w = (lambda a: (lambda t: t.astype(jnp.bfloat16) if jnp.issubdtype(t.dtype, jnp.floating) else t)(jnp.asarray(a)))
    def _A_setup():
        B, H, Sq, Sk, D, M = 1, 16, 2048, 2048, 256, 448
        Dc = 4 * D
        return {
            "x": _w((lambda *s: _rng.normal(s) * 0.05)(B, Sq, M)),
            "c_kv": _w((lambda *s: _rng.normal(s) * 0.05)(B, Sk, Dc)),
            "w_q": _w((lambda *s: _rng.normal(s) * 0.05)(M, H, D) * (M ** -0.5)),
            "w_uk": _w((lambda *s: _rng.normal(s) * 0.05)(Dc, H, D) * (Dc ** -0.5)),
            "w_uv": _w((lambda *s: _rng.normal(s) * 0.05)(Dc, H, D) * (Dc ** -0.5)),
            "w_o": _w((lambda *s: _rng.normal(s) * 0.05)(H, D, M) * ((H * D) ** -0.5)),
        }
    _A_in = _A_setup()

    def _B_setup():
        B, S, D, F, C = 1, 2048, 448, 1792, 2
        return {
            "x": _w((lambda *s: _rng.normal(s) * 0.05)(B, S, D)),
            "w_r": _w((lambda *s: _rng.normal(s) * 0.05)(D)),
            "w_gate": _w((lambda *s: _rng.normal(s) * 0.05)(D, F)),
            "w_up": _w((lambda *s: _rng.normal(s) * 0.05)(D, F)),
            "w_down": _w((lambda *s: _rng.normal(s) * 0.05)(F, D)),
        }
    _B_in = _B_setup()

    return {
        "A_x": _A_in["x"],
        "A_c_kv": _A_in["c_kv"],
        "A_w_q": _A_in["w_q"],
        "A_w_uk": _A_in["w_uk"],
        "A_w_uv": _A_in["w_uv"],
        "A_w_o": _A_in["w_o"],
        "B_x": _B_in["x"],
        "B_w_r": _B_in["w_r"],
        "B_w_gate": _B_in["w_gate"],
        "B_w_up": _B_in["w_up"],
        "B_w_down": _B_in["w_down"],
        "gate_w": _w((lambda *s: _rng.normal(s) * 0.05)(448)),
    }

def reference(A_x, A_c_kv, A_w_q, A_w_uk, A_w_uv, A_w_o, B_x, B_w_r, B_w_gate, B_w_up, B_w_down, gate_w):
    def _A_ref(x, c_kv, w_q, w_uk, w_uv, w_o):
        B, Sq, M = x.shape[0], x.shape[1], x.shape[2]
        Sk = c_kv.shape[1]
        H, D = w_q.shape[1], w_q.shape[2]
        q = jnp.einsum("bqm,mhd->bhqd", x, w_q)
        k = jnp.einsum("bkc,chd->bhkd", c_kv, w_uk)
        v = jnp.einsum("bkc,chd->bhkd", c_kv, w_uv)
        scores = jnp.einsum("bhqd,bhkd->bhqk", q, k) * (D ** -0.5)
        off = Sk - Sq
        qi = jnp.arange(Sq)[:, None]
        kj = jnp.arange(Sk)[None, :]
        cmask = kj <= (qi + off)
        scores = jnp.where(cmask[None, None], scores, -1e9)
        p = _softmax(scores, axis=-1)
        ctx = jnp.einsum("bhqk,bhkd->bhqd", p, v)
        return jnp.einsum("bhqd,hdm->bqm", ctx, w_o)

    def _B_ref(x, w_r, w_gate, w_up, w_down):
        B, S, D = x.shape
        C = 2
        r = x @ w_r
        idx = jnp.argsort(-r, axis=-1)[:, :C]
        idx_e = jnp.repeat(idx.reshape(B, C, 1), D, axis=2)
        x_sel = jnp.take_along_axis(x, idx_e, axis=1)
        g = _silu(x_sel @ w_gate)
        u = x_sel @ w_up
        y = (g * u) @ w_down
        r_sel = _sigmoid(jnp.take_along_axis(r, idx, axis=1))
        y = y * r_sel.reshape(B, C, 1)
        b_off = (jnp.arange(B) * S).reshape(B, 1)
        flat_idx = (idx + b_off).reshape(B * C)
        zero = (x * 0.0).reshape(B * S, D)
        upd = _scatter_add(zero, flat_idx, y.reshape(B * C, D), axis=0)
        return x + upd.reshape(B, S, D)

    x = A_x
    g = _sigmoid((x * gate_w).sum(-1, keepdims=True))
    a = _A_ref(x, A_c_kv, A_w_q, A_w_uk, A_w_uv, A_w_o)
    b = _B_ref(x, B_w_r, B_w_gate, B_w_up, B_w_down)
    return g * a + (1 - g) * b
```

```python
import functools
import math

import jax
import jax.numpy as jnp
import numpy as np
from jax import lax
from jax.experimental import pallas as pl
from jax.experimental.pallas import tpu as pltpu

_NT = (((1,), (1,)), ((), ()))
_BF = jnp.bfloat16
_F32 = jnp.float32
_LOG2E = math.log2(math.e)


def _dot(a, b):
    return jnp.dot(a, b, preferred_element_type=_F32)


def _dot_nt(a, b):
    return lax.dot_general(a, b, _NT, preferred_element_type=_F32)


def _split_pair(w):
    lo = lax.bitcast_convert_type(w << 16, _F32).astype(_BF)
    hi = lax.bitcast_convert_type(w & np.uint32(0xFFFF0000), _F32).astype(_BF)
    return lo, hi


def make(cfg):
    TQ = cfg.get("TQ", 128)
    PB = cfg.get("PB", 512)
    OB = cfg.get("OB", 512)
    LOOK = cfg.get("LOOK", 1)
    HPS = cfg.get("HPS", 2)

    def kernel(xt_hbm, c_hbm, wq_hbm, wk_hbm, wv_hbm, wot_hbm, wr_ref, wg_hbm, wu_hbm, wdt_hbm, gw_ref,
               out_hbm,
               xt_v, x_v, c_v, wq_v, wk_v, wv_v, wot_v, wg_v, wu_v, wdt_v, ctx_v, o_v,
               sem_in, sem_w, sem_o):
        M, S = xt_v.shape
        H, _, D = wot_v.shape
        NP = H // 2
        scale = (D ** -0.5) * _LOG2E
        neg = -1e9 * _LOG2E

        def w_copies(p, slot):
            return [
                pltpu.make_async_copy(src.bitcast(jnp.uint32).at[:, p, :], dst.at[slot], sem_w.at[i, slot])
                for i, (src, dst) in enumerate(((wq_hbm, wq_v), (wk_hbm, wk_v), (wv_hbm, wv_v)))
            ]

        cp_x = pltpu.make_async_copy(xt_hbm, xt_v, sem_in.at[0])
        cp_c = pltpu.make_async_copy(c_hbm, c_v, sem_in.at[1])
        cp_rest = [
            pltpu.make_async_copy(wot_hbm, wot_v, sem_in.at[2]),
            pltpu.make_async_copy(wg_hbm, wg_v, sem_in.at[3]),
            pltpu.make_async_copy(wu_hbm, wu_v, sem_in.at[4]),
            pltpu.make_async_copy(wdt_hbm, wdt_v, sem_in.at[5]),
        ]
        cp_x.start()
        for c in w_copies(0, 0):
            c.start()
        cp_c.start()
        cp_x.wait()
        x_v[...] = xt_v[...].T
        cp_c.wait()
        for c in cp_rest:
            c.start()

        row = lax.broadcasted_iota(jnp.int32, (TQ, TQ), 0)
        col = lax.broadcasted_iota(jnp.int32, (TQ, TQ), 1)
        tri = col <= row

        def head(h, wq, wk, wv):
            nb = S // PB
            q, k, v = [None] * nb, [None] * nb, [None] * nb

            def proj(b):
                rows = slice(b * PB, (b + 1) * PB)
                q[b] = (_dot(x_v[rows, :], wq) * scale).astype(_BF)
                cb = c_v[rows, :]
                k[b] = _dot(cb, wk).astype(_BF)
                v[b] = _dot(cb, wv).astype(_BF)

            def upto(lst, n):
                full, rem = divmod(n, PB)
                parts = list(lst[:full])
                if rem:
                    parts.append(lst[full][:rem])
                return parts[0] if len(parts) == 1 else jnp.concatenate(parts, axis=0)

            def qk(t):
                b, o = divmod(t * TQ, PB)
                n = (t + 1) * TQ
                return _dot_nt(q[b][o:o + TQ], upto(k, n))

            def pv(t, s):
                n = (t + 1) * TQ
                sd = jnp.where(tri, s[:, n - TQ:], neg)
                s = sd if t == 0 else jnp.concatenate([s[:, :n - TQ], sd], axis=1)
                m = jnp.max(s, axis=1, keepdims=True)
                p = jnp.exp2(s - m)
                l = jnp.sum(p, axis=1, keepdims=True)
                o = _dot(p.astype(_BF), upto(v, n))
                ctx_v[h, t * TQ:(t + 1) * TQ, :] = (o * (1.0 / l)).astype(_BF)

            nt = S // TQ
            done = 0
            pend = {}
            for t in range(nt + LOOK):
                if t < nt:
                    need = ((t + 1) * TQ + PB - 1) // PB
                    while done < need:
                        proj(done)
                        done += 1
                    pend[t] = qk(t)
                if t >= LOOK:
                    pv(t - LOOK, pend.pop(t - LOOK))

        def pair(p, _):
            slot = p % 2
            for c in w_copies(p, slot):
                c.wait()

            @pl.when(p + 1 < NP)
            def _():
                for c in w_copies(p + 1, 1 - slot):
                    c.start()

            wq = _split_pair(wq_v[slot])
            wk = _split_pair(wk_v[slot])
            wv = _split_pair(wv_v[slot])
            for i in range(2):
                head(2 * p + i, wq[i], wk[i], wv[i])

        lax.fori_loop(0, NP, pair, None)

        for c in cp_rest:
            c.wait()

        wr = wr_ref[...].astype(_F32).reshape(1, M)
        gw = gw_ref[...].astype(_F32).reshape(1, M)
        sub = lax.broadcasted_iota(jnp.int32, (16, M), 0)
        rg = _dot(jnp.where(sub == 0, wr, jnp.where(sub == 1, gw, 0.0)).astype(_BF), xt_v[...])
        r = rg[0:1].astype(_BF).astype(_F32)
        gate = jax.nn.sigmoid(rg[1:2])
        lane = lax.broadcasted_iota(jnp.int32, (1, S), 1)
        key = jnp.where(r != r, -jnp.inf, r)
        m1 = jnp.max(key, axis=1, keepdims=True)
        i1 = jnp.min(jnp.where(key == m1, lane, S), axis=1, keepdims=True)
        key2 = jnp.where(lane == i1, -jnp.inf, key)
        m2 = jnp.max(key2, axis=1, keepdims=True)
        i2 = jnp.min(jnp.where((key2 == m2) & (lane != i1), lane, S), axis=1, keepdims=True)
        sub_s = lax.broadcasted_iota(jnp.int32, (16, S), 0)
        lane_s = lax.broadcasted_iota(jnp.int32, (16, S), 1)
        onehot = jnp.where(((sub_s == 0) & (lane_s == i1)) | ((sub_s == 1) & (lane_s == i2)), 1.0, 0.0).astype(_BF)
        xs = _dot(onehot, x_v[...]).astype(_BF)
        a = _dot(xs, wg_v[...])
        u = _dot(xs, wu_v[...])
        hmid = (a * jax.nn.sigmoid(a) * u).astype(_BF)
        y = _dot_nt(hmid, wdt_v[...])
        sub1 = lax.broadcasted_iota(jnp.int32, (16, 1), 0)
        y = y * jax.nn.sigmoid(jnp.where(sub1 == 0, m1, m2))
        yt = jnp.concatenate([y, jnp.zeros((112, M), _F32)], axis=0).T
        y1, y2 = yt[:, 0:1], yt[:, 1:2]

        outs = []
        for b in range(S // OB):
            cols = slice(b * OB, (b + 1) * OB)
            acc = None
            for h in range(H):
                d = _dot_nt(wot_v[h], ctx_v[h, cols, :])
                acc = d if acc is None else acc + d
            xb = xt_v[:, cols].astype(_F32)
            lb = lane[:, cols]
            upd = xb * 0.0 + jnp.where(lb == i1, y1, jnp.where(lb == i2, y2, 0.0))
            g = gate[:, cols]
            o_v[:, cols] = (g * acc + (1.0 - g) * (xb + upd)).astype(o_v.dtype)
            cp = pltpu.make_async_copy(o_v.at[:, cols], out_hbm.at[:, cols], sem_o.at[b])
            cp.start()
            outs.append(cp)
        for cp in outs:
            cp.wait()

    def fn(A_x, A_c_kv, A_w_q, A_w_uk, A_w_uv, A_w_o, B_x, B_w_r, B_w_gate, B_w_up, B_w_down, gate_w):
        del B_x
        _, S, M = A_x.shape
        Dc = A_c_kv.shape[2]
        H, D = A_w_q.shape[1:]
        F = B_w_gate.shape[1]
        hbm = pl.BlockSpec(memory_space=pl.ANY)
        vmem = pl.BlockSpec(memory_space=pltpu.VMEM)
        out_t = pl.pallas_call(
            kernel,
            out_shape=jax.ShapeDtypeStruct((M, S), A_x.dtype),
            in_specs=[hbm, hbm, hbm, hbm, hbm, hbm, vmem, hbm, hbm, hbm, vmem],
            out_specs=hbm,
            scratch_shapes=[
                pltpu.VMEM((M, S), _BF),
                pltpu.VMEM((S, M), _BF),
                pltpu.VMEM((S, Dc), _BF),
                pltpu.VMEM((2, M, D), jnp.uint32),
                pltpu.VMEM((2, Dc, D), jnp.uint32),
                pltpu.VMEM((2, Dc, D), jnp.uint32),
                pltpu.VMEM((H, M, D), _BF),
                pltpu.VMEM((M, F), _BF),
                pltpu.VMEM((M, F), _BF),
                pltpu.VMEM((M, F), _BF),
                pltpu.VMEM((H, S, D), _BF),
                pltpu.VMEM((M, S), _BF),
                pltpu.SemaphoreType.DMA((6,)),
                pltpu.SemaphoreType.DMA((3, 2)),
                pltpu.SemaphoreType.DMA((S // OB,)),
            ],
            compiler_params=pltpu.CompilerParams(vmem_limit_bytes=110 * 2**20, flags=cfg.get("flags")),
            name=cfg.get("name", "gm"),
        )(A_x[0].T, A_c_kv[0], A_w_q, A_w_uk, A_w_uv, A_w_o.transpose(0, 2, 1), B_w_r, B_w_gate, B_w_up,
          B_w_down.T, gate_w)
        return out_t.T[None]

    return fn


_IMPL = make({})


@jax.jit
def pallas_gated_mix__compressed_kv_cla__moe_arch_mod__prompt_kernel(
    A_x, A_c_kv, A_w_q, A_w_uk, A_w_uv, A_w_o, B_x, B_w_r, B_w_gate, B_w_up, B_w_down, gate_w
):
    return _IMPL(A_x, A_c_kv, A_w_q, A_w_uk, A_w_uv, A_w_o, B_x, B_w_r, B_w_gate, B_w_up, B_w_down, gate_w)
```

```python
import functools
import math

import jax
import jax.numpy as jnp
import numpy as np
from jax import lax
from jax.experimental import pallas as pl
from jax.experimental.pallas import tpu as pltpu

_NT = (((1,), (1,)), ((), ()))
_BF = jnp.bfloat16
_F32 = jnp.float32
_LOG2E = math.log2(math.e)


def _dot(a, b):
    return jnp.dot(a, b, preferred_element_type=_F32)


def _dot_nt(a, b):
    return lax.dot_general(a, b, _NT, preferred_element_type=_F32)


def _pick_head(w, shift):
    return lax.bitcast_convert_type((w >> shift) << 16, _F32).astype(_BF)


def make(cfg):
    TQ = cfg.get("TQ", 128)
    PB = cfg.get("PB", 512)
    OB = cfg.get("OB", 512)
    LOOK = cfg.get("LOOK", 1)
    OLAG = cfg.get("OLAG", 1)
    DESC = cfg.get("DESC", 1)
    SCOPES = cfg.get("SCOPES", 0)

    def scope(name):
        import contextlib
        return jax.named_scope(name) if SCOPES else contextlib.nullcontext()

    def kernel(xt_hbm, c_hbm, wq_hbm, wk_hbm, wv_hbm, wot_hbm, wr_ref, wg_hbm, wu_hbm, wdt_hbm, gw_ref,
               out_hbm,
               xt_v, x_v, c_v, wq_v, wk_v, wv_v, wot_v, wg_v, wu_v, wdt_v, acc_v, gate_v, o_v,
               sem_in, sem_w, sem_o):
        M, S = xt_v.shape
        H, _, D = wot_v.shape
        NH = cfg.get("NH", H)
        scale = (D ** -0.5) * _LOG2E
        neg = -1e9 * _LOG2E

        def w_copies(p, slot):
            return [
                pltpu.make_async_copy(src.bitcast(jnp.uint32).at[:, p, :], dst.at[slot], sem_w.at[i, slot])
                for i, (src, dst) in enumerate(((wq_hbm, wq_v), (wk_hbm, wk_v), (wv_hbm, wv_v)))
            ]

        cp_x = pltpu.make_async_copy(xt_hbm, xt_v, sem_in.at[0])
        cp_c = pltpu.make_async_copy(c_hbm, c_v, sem_in.at[1])
        cp_wo = pltpu.make_async_copy(wot_hbm, wot_v, sem_in.at[2])
        cp_ffn = [
            pltpu.make_async_copy(wg_hbm, wg_v, sem_in.at[3]),
            pltpu.make_async_copy(wu_hbm, wu_v, sem_in.at[4]),
            pltpu.make_async_copy(wdt_hbm, wdt_v, sem_in.at[5]),
        ]

        def out_copy(b):
            cols = slice(b * OB, (b + 1) * OB)
            return pltpu.make_async_copy(o_v.at[:, cols], out_hbm.at[:, cols], sem_o.at[b])

        cp_x.start()
        for c in w_copies(0, 0):
            c.start()
        cp_c.start()
        cp_wo.start()
        with scope("waitx"):
            cp_x.wait()
        x_v[...] = xt_v[...].T
        acc_v[...] = jnp.zeros_like(acc_v)
        wr = wr_ref[...].astype(_F32).reshape(1, M)
        gw = gw_ref[...].astype(_F32).reshape(1, M)
        sub = lax.broadcasted_iota(jnp.int32, (16, M), 0)
        rg = _dot(jnp.where(sub == 0, wr, jnp.where(sub == 1, gw, 0.0)).astype(_BF), xt_v[...])
        gate_v[...] = rg[0:8]
        with scope("waitc"):
            cp_c.wait()
            cp_wo.wait()
        for c in cp_ffn:
            c.start()

        def ffn():
            for c in cp_ffn:
                c.wait()
            r = gate_v[0:1, :].astype(_BF).astype(_F32)
            gate = jax.nn.sigmoid(gate_v[1:2, :])
            lane = lax.broadcasted_iota(jnp.int32, (1, S), 1)
            key = jnp.where(r != r, -jnp.inf, r)
            m1 = jnp.max(key, axis=1, keepdims=True)
            i1 = jnp.min(jnp.where(key == m1, lane, S), axis=1, keepdims=True)
            key2 = jnp.where(lane == i1, -jnp.inf, key)
            m2 = jnp.max(key2, axis=1, keepdims=True)
            i2 = jnp.min(jnp.where((key2 == m2) & (lane != i1), lane, S), axis=1, keepdims=True)
            sub_s = lax.broadcasted_iota(jnp.int32, (16, S), 0)
            lane_s = lax.broadcasted_iota(jnp.int32, (16, S), 1)
            onehot = jnp.where(((sub_s == 0) & (lane_s == i1)) | ((sub_s == 1) & (lane_s == i2)), 1.0, 0.0).astype(_BF)
            xs = _dot(onehot, x_v[...]).astype(_BF)
            a = _dot(xs, wg_v[...])
            u = _dot(xs, wu_v[...])
            hmid = (a * jax.nn.sigmoid(a) * u).astype(_BF)
            y = _dot_nt(hmid, wdt_v[...])
            sub1 = lax.broadcasted_iota(jnp.int32, (16, 1), 0)
            y = y * jax.nn.sigmoid(jnp.where(sub1 == 0, m1, m2))
            yt = jnp.concatenate([y, jnp.zeros((112, M), _F32)], axis=0).T
            y1, y2 = yt[:, 0:1], yt[:, 1:2]
            xb = xt_v[...].astype(_F32)
            upd = xb * 0.0 + jnp.where(lane == i1, y1, jnp.where(lane == i2, y2, 0.0))
            for b in range(S // OB):
                cols = slice(b * OB, (b + 1) * OB)
                g = gate[:, cols]
                o_v[:, cols] = (g * acc_v[:, cols] + (1.0 - g) * (xb + upd)[:, cols]).astype(o_v.dtype)
                out_copy(b).start()
            for b in range(S // OB):
                out_copy(b).wait()

        def head(h, _):
            slot = (h // 2) % 2
            odd = h % 2

            @pl.when(odd == 0)
            def _():
                for c in w_copies(h // 2, slot):
                    c.wait()

            @pl.when((odd == 0) & (h + 2 < NH))
            def _():
                for c in w_copies(h // 2 + 1, 1 - slot):
                    c.start()

            shift = (odd * 16).astype(jnp.uint32)
            wq = _pick_head(wq_v[slot], shift)
            wk = _pick_head(wk_v[slot], shift)
            wv = _pick_head(wv_v[slot], shift)
            wot = wot_v[h]

            row = lax.broadcasted_iota(jnp.int32, (TQ, TQ), 0)
            col = lax.broadcasted_iota(jnp.int32, (TQ, TQ), 1)
            tri = col <= row

            nb = S // PB
            q, k, v = [None] * nb, [None] * nb, [None] * nb

            def proj(b):
                rows = slice(b * PB, (b + 1) * PB)
                q[b] = (_dot(x_v[rows, :], wq) * scale).astype(_BF)
                cb = c_v[rows, :]
                k[b] = _dot(cb, wk).astype(_BF)
                v[b] = _dot(cb, wv).astype(_BF)

            def upto(lst, n):
                full, rem = divmod(n, PB)
                parts = list(lst[:full])
                if rem:
                    parts.append(lst[full][:rem])
                return parts[0] if len(parts) == 1 else jnp.concatenate(parts, axis=0)

            def qk(t):
                b, o = divmod(t * TQ, PB)
                n = (t + 1) * TQ
                return _dot_nt(q[b][o:o + TQ], upto(k, n))

            def pv(t, s):
                n = (t + 1) * TQ
                sd = jnp.where(tri, s[:, n - TQ:], neg)
                s = sd if t == 0 else jnp.concatenate([s[:, :n - TQ], sd], axis=1)
                m = jnp.max(s, axis=1, keepdims=True)
                p = jnp.exp2(s - m)
                l = jnp.sum(p, axis=1, keepdims=True)
                o = _dot(p.astype(_BF), upto(v, n))
                return (o * (1.0 / l)).astype(_BF)

            def oproj(t, ctx):
                cols = slice(t * TQ, (t + 1) * TQ)
                acc_v[:, cols] += _dot_nt(wot, ctx)

            nt = S // TQ
            order = list(range(nt))[::-1] if DESC else list(range(nt))
            done = 0
            pend, ctxs = {}, {}
            for i in range(nt + LOOK + OLAG):
                if i < nt:
                    t = order[i]
                    need = ((t + 1) * TQ + PB - 1) // PB
                    while done < need:
                        proj(done)
                        done += 1
                    pend[t] = qk(t)
                if LOOK <= i < nt + LOOK:
                    t = order[i - LOOK]
                    ctxs[t] = pv(t, pend.pop(t))
                if i >= LOOK + OLAG:
                    t = order[i - LOOK - OLAG]
                    oproj(t, ctxs.pop(t))

        with scope("loop"):
            lax.fori_loop(0, NH, head, None)
        with scope("ffn"):
            ffn()

    def fn(A_x, A_c_kv, A_w_q, A_w_uk, A_w_uv, A_w_o, B_x, B_w_r, B_w_gate, B_w_up, B_w_down, gate_w):
        del B_x
        _, S, M = A_x.shape
        Dc = A_c_kv.shape[2]
        H, D = A_w_q.shape[1:]
        F = B_w_gate.shape[1]
        hbm = pl.BlockSpec(memory_space=pl.ANY)
        vmem = pl.BlockSpec(memory_space=pltpu.VMEM)
        out_t = pl.pallas_call(
            kernel,
            out_shape=jax.ShapeDtypeStruct((M, S), A_x.dtype),
            in_specs=[hbm, hbm, hbm, hbm, hbm, hbm, vmem, hbm, hbm, hbm, vmem],
            out_specs=hbm,
            scratch_shapes=[
                pltpu.VMEM((M, S), _BF),
                pltpu.VMEM((S, M), _BF),
                pltpu.VMEM((S, Dc), _BF),
                pltpu.VMEM((2, M, D), jnp.uint32),
                pltpu.VMEM((2, Dc, D), jnp.uint32),
                pltpu.VMEM((2, Dc, D), jnp.uint32),
                pltpu.VMEM((H, M, D), _BF),
                pltpu.VMEM((M, F), _BF),
                pltpu.VMEM((M, F), _BF),
                pltpu.VMEM((M, F), _BF),
                pltpu.VMEM((M, S), _F32),
                pltpu.VMEM((8, S), _F32),
                pltpu.VMEM((M, S), _BF),
                pltpu.SemaphoreType.DMA((6,)),
                pltpu.SemaphoreType.DMA((3, 2)),
                pltpu.SemaphoreType.DMA((S // OB,)),
            ],
            compiler_params=pltpu.CompilerParams(vmem_limit_bytes=110 * 2**20, flags=cfg.get("flags")),
            name=cfg.get("name", "gm"),
        )(A_x[0].T, A_c_kv[0], A_w_q, A_w_uk, A_w_uv, A_w_o.transpose(0, 2, 1), B_w_r, B_w_gate, B_w_up,
          B_w_down.T, gate_w)
        return out_t.T[None]

    return fn


_IMPL = make({'LOOK': 2, 'OLAG': 4})


@jax.jit
def pallas_gated_mix__compressed_kv_cla__moe_arch_mod__prompt_kernel(
    A_x, A_c_kv, A_w_q, A_w_uk, A_w_uv, A_w_o, B_x, B_w_r, B_w_gate, B_w_up, B_w_down, gate_w
):
    return _IMPL(A_x, A_c_kv, A_w_q, A_w_uk, A_w_uv, A_w_o, B_x, B_w_r, B_w_gate, B_w_up, B_w_down, gate_w)
```

```python
import contextlib
import math

import jax
import jax.numpy as jnp
import numpy as np
from jax import lax
from jax.experimental import pallas as pl
from jax.experimental.pallas import tpu as pltpu

_NT = (((1,), (1,)), ((), ()))
_BF = jnp.bfloat16
_F32 = jnp.float32
_LOG2E = math.log2(math.e)
_LANES = 128


def _dot(a, b):
    return jnp.dot(a, b, preferred_element_type=_F32)


def _dot_nt(a, b):
    return lax.dot_general(a, b, _NT, preferred_element_type=_F32)


def _pick_head(w, shift):
    return lax.bitcast_convert_type((w >> shift) << 16, _F32).astype(_BF)


def _split_pair(w):
    lo = lax.bitcast_convert_type(w << 16, _F32).astype(_BF)
    hi = lax.bitcast_convert_type(w & np.uint32(0xFFFF0000), _F32).astype(_BF)
    return lo, hi


def _column(vec):
    n = vec.shape[0]
    return jnp.broadcast_to(vec.astype(_F32).reshape(1, n), (_LANES, n)).T


def make(cfg):
    TQ = cfg.get("TQ", 128)
    PB = cfg.get("PB", 512)
    XB = cfg.get("XB", 512)
    QB = cfg.get("QB", 512)
    OB = cfg.get("OB", 256)
    LOOK = cfg.get("LOOK", 2)
    OLAG = cfg.get("OLAG", 4)
    DESC = cfg.get("DESC", 1)
    FPOS = cfg.get("FPOS", 4)
    RPOS = cfg.get("RPOS", 0)
    DORD2 = cfg.get("DORD2", 0)
    XPOS = cfg.get("XPOS", 2)
    DORD = cfg.get("DORD", 0)
    SCOPES = cfg.get("SCOPES", 0)

    def scope(name):
        return jax.named_scope(name) if SCOPES else contextlib.nullcontext()

    def kernel(xt_hbm, c_hbm, wq_hbm, wk_hbm, wv_hbm, wot_hbm, wr_hbm, wg_hbm, wu_hbm, wdt_hbm, gw_hbm,
               out_hbm,
               xt_v, x_v, q_v, c_v, wq_v, wk_v, wv_v, wkb_v, wvb_v, wot_v, wr_v, gw_v, wg_v, wu_v, wdt_v,
               acc_v, row_v, wcol_v, xs_v, y_v, o_v,
               idx_s, sem_x, sem_q, sem_w, sem_m, sem_o):
        M, S = xt_v.shape
        H, _, D = q_v.shape
        F = wg_v.shape[1]
        NH = cfg.get("NH", H)
        NF = F // _LANES
        scale = (D ** -0.5) * _LOG2E
        neg = -1e9 * _LOG2E

        def wq_copy(p):
            return pltpu.make_async_copy(wq_hbm.bitcast(jnp.uint32).at[:, p, :], wq_v.at[p], sem_q.at[p])

        def pair_copies(p):
            return [
                pltpu.make_async_copy(wk_hbm.bitcast(jnp.uint32).at[:, p, :], wk_v.at[p], sem_w.at[3 * p]),
                pltpu.make_async_copy(wv_hbm.bitcast(jnp.uint32).at[:, p, :], wv_v.at[p], sem_w.at[3 * p + 1]),
                pltpu.make_async_copy(wot_hbm.at[pl.ds(2 * p, 2)], wot_v.at[pl.ds(2 * p, 2)], sem_w.at[3 * p + 2]),
            ]

        def x_copy(b):
            cols = slice(b * XB, (b + 1) * XB)
            return pltpu.make_async_copy(xt_hbm.at[:, cols], xt_v.at[:, cols], sem_x.at[b])

        def out_copy(b):
            cols = slice(b * OB, (b + 1) * OB)
            return pltpu.make_async_copy(o_v.at[:, cols], out_hbm.at[:, cols], sem_o.at[b])

        misc = [pltpu.make_async_copy(s, d, sem_m.at[i]) for i, (s, d) in enumerate((
            (wr_hbm, wr_v), (gw_hbm, gw_v), (c_hbm, c_v), (wg_hbm, wg_v), (wu_hbm, wu_v), (wdt_hbm, wdt_v)))]

        def token_tile(i):
            start = pl.multiple_of((i // _LANES) * _LANES, _LANES)
            hit = lax.broadcasted_iota(jnp.int32, (1, _LANES), 1) == i - start
            return pl.ds(start, _LANES), hit

        def q_pair(p, rows, x):
            for i, w in enumerate(_split_pair(wq_v[p])):
                q_v[2 * p + i, rows, :] = (_dot(x, w) * scale).astype(_BF)

        def x_transpose(b):
            x_v[b * XB:(b + 1) * XB, :] = xt_v[:, b * XB:(b + 1) * XB].T

        def token_stats(cols):
            xb = xt_v[:, cols].astype(_F32)
            r = jnp.sum(xb * wcol_v[0], axis=0, keepdims=True).astype(_BF).astype(_F32)
            g = jax.nn.sigmoid(jnp.sum(xb * wcol_v[1], axis=0, keepdims=True))
            row_v[0:1, cols] = r
            row_v[1:2, cols] = g
            row_v[2:3, cols] = jax.nn.sigmoid(r) * (1.0 - g)
            acc_v[:, cols] = (1.0 - g) * (xb + xb * 0.0)

        def route():
            r = row_v[0:1, :]
            lane = lax.broadcasted_iota(jnp.int32, (1, S), 1)
            key = jnp.where(r != r, -jnp.inf, r)
            i1 = jnp.min(jnp.where(key == jnp.max(key), lane, S - 1))
            key = jnp.where(lane == i1, -jnp.inf, key)
            i2 = jnp.min(jnp.where((key == jnp.max(key)) & (lane != i1), lane, S - 1))
            idx_s[0] = i1
            idx_s[1] = i2
            for e, i in enumerate((i1, i2)):
                cols, hit = token_tile(i)
                xe = jnp.sum(jnp.where(hit, xt_v[:, cols].astype(_F32), 0.0), axis=1, keepdims=True)
                xs_v[e] = jnp.broadcast_to(xe, (M, _LANES))

        nx = S // XB
        misc[0].start()
        misc[1].start()
        wq_copy(0).start()
        x_copy(0).start()
        if DORD < 2:
            for b in range(1, nx):
                x_copy(b).start()
        if DORD < 1:
            for p in range(1, H // 2):
                wq_copy(p).start()

        def start_rest():
            for c in pair_copies(0) + misc[2:]:
                c.start()
            for p in range(1, NH // 2):
                for c in pair_copies(p):
                    c.start()

        if DORD2 == 0:
            start_rest()
        y_v[...] = jnp.zeros_like(y_v)
        misc[0].wait()
        misc[1].wait()
        wcol_v[0] = _column(wr_v[...])
        wcol_v[1] = _column(gw_v[...])
        with scope("wait0"):
            wq_copy(0).wait()
            x_copy(0).wait()
        if DORD >= 2:
            for b in range(1, nx):
                x_copy(b).start()
        if DORD >= 1:
            for p in range(1, H // 2):
                wq_copy(p).start()
        x_transpose(0)
        q_pair(0, slice(0, XB), x_v[0:XB, :])
        if nx > 1:
            with scope("wait1"):
                for b in range(1, nx):
                    x_copy(b).wait()
            if DORD2 == 1:
                start_rest()
            for b in range(1, nx):
                x_transpose(b)
                q_pair(0, slice(b * XB, (b + 1) * XB), x_v[b * XB:(b + 1) * XB, :])
        with scope("wait2"):
            for p in range(1, H // 2):
                wq_copy(p).wait()
        if DORD2 == 2:
            start_rest()

        def q_rest(b, _):
            rows = pl.ds(pl.multiple_of(b * QB, QB), QB)
            x = x_v[rows, :]
            tiles = list(range(QB // _LANES))
            for p in range(1, H // 2):
                q_pair(p, rows, x)
                todo = -(-len(tiles) // (H // 2 - p))
                for t in tiles[:todo]:
                    token_stats(pl.ds(pl.multiple_of(b * QB + t * _LANES, _LANES), _LANES))
                tiles = tiles[todo:]

        with scope("qloop"):
            lax.fori_loop(0, S // QB, q_rest, None)
        with scope("wait3"):
            for c in pair_copies(0) + misc[2:]:
                c.wait()
        wkb_v[...] = _split_pair(wk_v[0])[0]
        wvb_v[...] = _split_pair(wv_v[0])[0]

        def ffn_chunk(h):
            cols = pl.ds(pl.multiple_of(jnp.minimum(h, NF - 1) * _LANES, _LANES), _LANES)
            wg = wg_v[:, cols].astype(_F32)
            wu = wu_v[:, cols].astype(_F32)
            wd = wdt_v[:, cols].astype(_F32)
            for e in range(2):
                xe = xs_v[e]
                a = jnp.sum(wg * xe, axis=0, keepdims=True)
                u = jnp.sum(wu * xe, axis=0, keepdims=True)
                y_v[e] += wd * (a * jax.nn.sigmoid(a) * u)

        def ffn_scatter():
            for e in range(2):
                cols, hit = token_tile(idx_s[e])
                ye = jnp.sum(y_v[e], axis=1, keepdims=True)
                acc_v[:, cols] += jnp.where(hit, ye * row_v[2:3, cols], 0.0)

        def head(h, _):
            odd = h % 2

            @pl.when((odd == 1) & (h + 1 < NH))
            def _():
                for c in pair_copies(h // 2 + 1):
                    c.wait()

            @pl.when(h == NF)
            def _():
                ffn_scatter()

            row = lax.broadcasted_iota(jnp.int32, (TQ, TQ), 0)
            col = lax.broadcasted_iota(jnp.int32, (TQ, TQ), 1)
            tri = col <= row

            nb = S // PB
            k, v = [], []
            for b in range(nb):
                k.append(_dot(c_v[b * PB:(b + 1) * PB, :], wkb_v[...]).astype(_BF))
                if b == RPOS:
                    route()
                if b == FPOS:
                    ffn_chunk(h)
            nslot = jnp.minimum(h + 1, NH - 1) // 2
            nshift = ((1 - odd) * 16).astype(jnp.uint32)
            for b in range(nb):
                v.append(_dot(c_v[b * PB:(b + 1) * PB, :], wvb_v[...]).astype(_BF))
                if b + nb == FPOS:
                    ffn_chunk(h)
                if b == XPOS:
                    wkb_v[...] = _pick_head(wk_v[nslot], nshift)
            wvb_v[...] = _pick_head(wv_v[nslot], nshift)
            wot = wot_v[h]

            def upto(lst, n):
                full, rem = divmod(n, PB)
                parts = list(lst[:full])
                if rem:
                    parts.append(lst[full][:rem])
                return parts[0] if len(parts) == 1 else jnp.concatenate(parts, axis=0)

            def qk(t):
                return _dot_nt(q_v[h, t * TQ:(t + 1) * TQ, :], upto(k, (t + 1) * TQ))

            def pv(t, s):
                n = (t + 1) * TQ
                sd = jnp.where(tri, s[:, n - TQ:], neg)
                s = sd if t == 0 else jnp.concatenate([s[:, :n - TQ], sd], axis=1)
                m = jnp.max(s, axis=1, keepdims=True)
                p = jnp.exp2(s - m)
                l = jnp.sum(p, axis=1, keepdims=True)
                o = _dot(p.astype(_BF), upto(v, n))
                return (o * (1.0 / l)).astype(_BF)

            stored = set()

            def oproj(t, ctx):
                cols = slice(t * TQ, (t + 1) * TQ)
                tot = acc_v[:, cols] + row_v[1:2, cols] * _dot_nt(wot, ctx)
                acc_v[:, cols] = tot
                o_v[:, cols] = tot.astype(o_v.dtype)
                stored.add(t)
                b = t * TQ // OB
                if all(u in stored for u in range(b * OB // TQ, (b + 1) * OB // TQ)):
                    pl.when(h == NH - 1)(lambda: out_copy(b).start())

            nt = S // TQ
            order = cfg.get("ORDER") or (list(range(nt))[::-1] if DESC else list(range(nt)))
            pend, ctxs = {}, {}
            for i in range(nt + LOOK + OLAG):
                if i < nt:
                    t = order[i]
                    pend[t] = qk(t)
                if LOOK <= i < nt + LOOK:
                    t = order[i - LOOK]
                    ctxs[t] = pv(t, pend.pop(t))
                if i >= LOOK + OLAG:
                    t = order[i - LOOK - OLAG]
                    oproj(t, ctxs.pop(t))

        with scope("loop"):
            lax.fori_loop(0, NH, head, None)
        with scope("tail"):
            for b in range(S // OB):
                out_copy(b).wait()

    def fn(A_x, A_c_kv, A_w_q, A_w_uk, A_w_uv, A_w_o, B_x, B_w_r, B_w_gate, B_w_up, B_w_down, gate_w):
        del B_x
        _, S, M = A_x.shape
        Dc = A_c_kv.shape[2]
        H, D = A_w_q.shape[1:]
        F = B_w_gate.shape[1]
        hbm = pl.BlockSpec(memory_space=pltpu.HBM)
        dma = pltpu.SemaphoreType.DMA
        out_t = pl.pallas_call(
            kernel,
            out_shape=jax.ShapeDtypeStruct((M, S), A_x.dtype),
            in_specs=[hbm] * 11,
            out_specs=hbm,
            scratch_shapes=[
                pltpu.VMEM((M, S), _BF),
                pltpu.VMEM((S, M), _BF),
                pltpu.VMEM((H, S, D), _BF),
                pltpu.VMEM((S, Dc), _BF),
                pltpu.VMEM((H // 2, M, D), jnp.uint32),
                pltpu.VMEM((H // 2, Dc, D), jnp.uint32),
                pltpu.VMEM((H // 2, Dc, D), jnp.uint32),
                pltpu.VMEM((Dc, D), _BF),
                pltpu.VMEM((Dc, D), _BF),
                pltpu.VMEM((H, M, D), _BF),
                pltpu.VMEM((M,), _BF),
                pltpu.VMEM((M,), _BF),
                pltpu.VMEM((M, F), _BF),
                pltpu.VMEM((M, F), _BF),
                pltpu.VMEM((M, F), _BF),
                pltpu.VMEM((M, S), _F32),
                pltpu.VMEM((8, S), _F32),
                pltpu.VMEM((2, M, _LANES), _F32),
                pltpu.VMEM((2, M, _LANES), _F32),
                pltpu.VMEM((2, M, _LANES), _F32),
                pltpu.VMEM((M, S), _BF),
                pltpu.SMEM((2,), jnp.int32),
                dma((S // XB,)),
                dma((H // 2,)),
                dma((3 * H // 2,)),
                dma((6,)),
                dma((S // OB,)),
            ],
            compiler_params=pltpu.CompilerParams(vmem_limit_bytes=110 * 2**20, flags=cfg.get("flags")),
            name=cfg.get("name", "gm"),
        )(A_x[0].T, A_c_kv[0], A_w_q, A_w_uk, A_w_uv, A_w_o.transpose(0, 2, 1), B_w_r, B_w_gate, B_w_up,
          B_w_down.T, gate_w)
        return out_t.T[None]

    return fn


_IMPL = make({})


@jax.jit
def pallas_gated_mix__compressed_kv_cla__moe_arch_mod__prompt_kernel(
    A_x, A_c_kv, A_w_q, A_w_uk, A_w_uv, A_w_o, B_x, B_w_r, B_w_gate, B_w_up, B_w_down, gate_w
):
    return _IMPL(A_x, A_c_kv, A_w_q, A_w_uk, A_w_uv, A_w_o, B_x, B_w_r, B_w_gate, B_w_up, B_w_down, gate_w)
```

```python
import contextlib
import math

import jax
import jax.numpy as jnp
import numpy as np
from jax import lax
from jax.experimental import pallas as pl
from jax.experimental.pallas import tpu as pltpu

_BF = jnp.bfloat16
_F32 = jnp.float32
_LOG2E = math.log2(math.e)
_LANES = 128


def _dot(a, b):
    return jnp.dot(a, b, preferred_element_type=_F32)


def _dot_nt(a, b):
    return lax.dot_general(a, b, (((1,), (1,)), ((), ())), preferred_element_type=_F32)


def _pick_head(w, odd):
    if isinstance(odd, int):
        bits = w & np.uint32(0xFFFF0000) if odd else w << 16
    else:
        bits = (w >> (odd * 16).astype(jnp.uint32)) << 16
    return lax.bitcast_convert_type(bits, _F32).astype(_BF)


def _column(vec):
    n = vec.shape[0]
    return jnp.broadcast_to(vec.astype(_F32).reshape(1, n), (_LANES, n)).T


def _schedule(nt, nb, cfg):
    if "SEQ" in cfg:
        return [(w[0], int(w[1:] or 0)) for w in cfg["SEQ"].split()]
    order = list(range(nt))[::-1]
    stages = [(w[0], int(w[1:])) for w in cfg.get("PIPE", "q0 p2 o6").split()]
    seq = [("k", b) for b in range(nb)] + [("v", b) for b in range(nb)]
    for n, op in reversed(list(zip(cfg.get("XP", (3, 0, 0, 6, 5)), "VRFSK"))):
        seq.insert(n * 2 * nb // 8 + 1, (op, 0))
    for i in range(nt + max(lag for _, lag in stages)):
        for op, lag in stages:
            if 0 <= i - lag < nt:
                seq.append((op, order[i - lag]))
    return seq


def make(cfg):
    TQ = _LANES
    PB = cfg.get("PB", 512)
    QB = cfg.get("QB", 512)
    SCOPES = cfg.get("SCOPES", 0)

    def scope(name):
        return jax.named_scope(name) if SCOPES else contextlib.nullcontext()

    def kernel(xt_hbm, c_hbm, wq_hbm, wk_hbm, wv_hbm, wot_hbm, wr_hbm, wg_hbm, wu_hbm, wdt_hbm, gw_hbm,
               out_hbm,
               xt_v, x_v, q_v, c_v, wq_v, wk_v, wv_v, wb_v, wot_v, wr_v, gw_v, wg_v, wu_v, wdt_v,
               acc_v, row_v, col_v, xs_v, y_v, o_v, idx_s, sems):
        M, S = xt_v.shape
        H, _, D = q_v.shape
        NP = H // 2
        NF = wg_v.shape[1] // _LANES
        scale = (D ** -0.5) * _LOG2E
        neg = -1e9 * _LOG2E

        def copy(src, dst, sem):
            return pltpu.make_async_copy(src, dst, sems.at[sem])

        def pair_copy(src, dst, p, sem):
            return copy(src.bitcast(jnp.uint32).at[:, p, :], dst.at[p], sem)

        def x_copy(a, b, sem):
            return copy(xt_hbm.at[:, a:b], xt_v.at[:, a:b], sem)

        def token_tile(i):
            start = pl.multiple_of((i // _LANES) * _LANES, _LANES)
            hit = lax.broadcasted_iota(jnp.int32, (1, _LANES), 1) == i - start
            return pl.ds(start, _LANES), hit

        def x_transpose(rows):
            x_v[rows, :] = xt_v[:, rows].T

        def q_head(h, rows):
            q_v[h, rows, :] = (_dot(x_v[rows, :], _pick_head(wq_v[h // 2], h % 2)) * scale).astype(_BF)

        def token_stats(cols):
            xb = xt_v[:, cols].astype(_F32)
            r = jnp.sum(xb * col_v[0], axis=0, keepdims=True).astype(_BF).astype(_F32)
            g = jax.nn.sigmoid(jnp.sum(xb * col_v[1], axis=0, keepdims=True))
            row_v[0:1, cols] = r
            row_v[1:2, cols] = g
            row_v[2:3, cols] = jax.nn.sigmoid(r) * (1.0 - g)
            acc_v[:, cols] = (1.0 - g) * (xb + xb * 0.0)

        def side_work(start):
            return [lambda t=t: token_stats(pl.ds(pl.multiple_of(start + t * _LANES, _LANES), _LANES))
                    for t in range(QB // _LANES)]

        def q_heads(heads, rows, work):
            for n, h in enumerate(heads):
                q_head(h, rows)
                if work and n in cfg.get("SW", (1, 3, 5, 7)):
                    work.pop(0)()

        def route():
            r = row_v[0:1, :]
            lane = lax.broadcasted_iota(jnp.int32, (1, S), 1)
            key = jnp.where(r != r, -jnp.inf, r)
            i1 = jnp.min(jnp.where(key == jnp.max(key), lane, S - 1))
            key = jnp.where(lane == i1, -jnp.inf, key)
            i2 = jnp.min(jnp.where((key == jnp.max(key)) & (lane != i1), lane, S - 1))
            idx_s[0] = i1
            idx_s[1] = i2
            for e, i in enumerate((i1, i2)):
                cols, hit = token_tile(i)
                xe = jnp.sum(jnp.where(hit, xt_v[:, cols].astype(_F32), 0.0), axis=1, keepdims=True)
                xs_v[e] = jnp.broadcast_to(xe, (M, _LANES))

        def ffn_chunk(h):
            cols = pl.ds(pl.multiple_of(jnp.minimum(h, NF - 1) * _LANES, _LANES), _LANES)
            wg = wg_v[:, cols].astype(_F32)
            wu = wu_v[:, cols].astype(_F32)
            wd = wdt_v[:, cols].astype(_F32)
            for e in range(2):
                xe = xs_v[e]
                a = jnp.sum(wg * xe, axis=0, keepdims=True)
                u = jnp.sum(wu * xe, axis=0, keepdims=True)
                y_v[e] += wd * (a * jax.nn.sigmoid(a) * u)

        def ffn_reduce(slot):
            for e in range(2):
                ye = jnp.sum(y_v[e], axis=1, keepdims=True)
                wb_v[slot, :M, e * _LANES:(e + 1) * _LANES] = jnp.broadcast_to(ye, (M, _LANES)).astype(_BF)

        def ffn_scatter():
            for e in range(2):
                cols, hit = token_tile(idx_s[e])
                ye = wb_v[3 - (NF - 1) % 2, :M, e * _LANES:(e + 1) * _LANES].astype(_F32)
                acc_v[:, cols] += jnp.where(hit, ye * row_v[2:3, cols], 0.0)

        x1, x2 = cfg.get("XG", (512, 1024))
        groups = [
            [copy(wr_hbm, wr_v, 0), copy(gw_hbm, gw_v, 0)],
            [pair_copy(wq_hbm, wq_v, 0, 1), x_copy(0, x1, 1)],
            [x_copy(x1, x2, 2)],
            [x_copy(x2, S, 3)] if x2 < S else [],
            [pair_copy(wq_hbm, wq_v, p, 4) for p in range(1, NP)],
            [copy(c_hbm, c_v, 5), pair_copy(wk_hbm, wk_v, 0, 5), pair_copy(wv_hbm, wv_v, 0, 5),
             copy(wot_hbm, wot_v, 5), copy(wg_hbm, wg_v, 5), copy(wu_hbm, wu_v, 5), copy(wdt_hbm, wdt_v, 5)],
            [pair_copy(wk_hbm, wk_v, p, 6) for p in range(1, NP)],
            [pair_copy(wv_hbm, wv_v, p, 7) for p in range(1, NP)],
        ]

        def wait_group(g):
            with scope("wait%d" % g):
                for c in groups[g]:
                    c.wait()

        early = cfg.get("EARLY", 8)
        for grp in groups[:early]:
            for c in grp:
                c.start()
        y_v[...] = jnp.zeros_like(y_v)
        wait_group(0)
        col_v[0] = _column(wr_v[...])
        col_v[1] = _column(gw_v[...])
        for grp in groups[early:]:
            for c in grp:
                c.start()

        spans = [slice(0, x1), slice(x1, x2)] + ([slice(x2, S)] if x2 < S else [])
        hold = cfg.get("HOLD", 1)
        for n, rows in enumerate(spans):
            wait_group(1 + n)
            if n and hold:
                q_head(1, spans[n - 1])
            x_transpose(rows)
            q_head(0, rows)
            if not hold or n == len(spans) - 1:
                q_head(1, rows)
        wait_group(4)

        def q_block(b, _):
            q_heads(range(2, H), pl.ds(pl.multiple_of(b * QB, QB), QB), side_work(b * QB))

        with scope("qloop"):
            lax.fori_loop(0, S // QB, q_block, None)
        wait_group(5)
        wb_v[0] = _pick_head(wk_v[0], 0)

        def head(h, _):
            odd = h % 2

            @pl.when(h == 1)
            def _():
                copy(wk_v.at[1:], wk_v.at[1:], 6).wait()
                copy(wv_v.at[1:], wv_v.at[1:], 7).wait()

            pl.when(h == NF)(ffn_scatter)

            tri = (lax.broadcasted_iota(jnp.int32, (TQ, TQ), 1)
                   <= lax.broadcasted_iota(jnp.int32, (TQ, TQ), 0))
            k, v, live, stored = [None] * (S // PB), [None] * (S // PB), {}, set()
            cuts = list(cfg.get("CUTS", range(0, S // TQ, 2))) + [S // TQ]

            def upto(blocks, n):
                full, rem = divmod(n, PB)
                parts = blocks[:full] + ([blocks[full][:rem]] if rem else [])
                return jnp.concatenate(parts, axis=0)

            for op, t in _schedule(S // TQ, S // PB, cfg):
                n = (t + 1) * TQ
                if op == "k":
                    k[t] = _dot(c_v[t * PB:(t + 1) * PB, :], wb_v[odd]).astype(_BF)
                elif op == "v":
                    v[t] = _dot(c_v[t * PB:(t + 1) * PB, :], wb_v[2 + odd]).astype(_BF)
                elif op == "V":
                    wb_v[2 + odd] = _pick_head(wv_v[h // 2], odd)
                elif op == "K":
                    wb_v[1 - odd] = _pick_head(wk_v[jnp.minimum(h + 1, H - 1) // 2], 1 - odd)
                elif op == "R":
                    route()
                elif op == "F":
                    ffn_chunk(h)
                elif op == "S":
                    ffn_reduce(3 - odd)
                elif op == "q":
                    s = _dot_nt(q_v[h, n - TQ:n, :], upto(k, n))
                    diag = jnp.where(tri, s[:, n - TQ:], neg)
                    s = jnp.concatenate([s[:, :n - TQ], diag], axis=1) if t else diag
                    p = jnp.exp2(s - jnp.max(s, axis=1, keepdims=True))
                    live[t] = p.astype(_BF), 1.0 / jnp.sum(p, axis=1, keepdims=True)
                elif op == "p":
                    p, inv = live[t]
                    live[t] = (_dot(p, upto(v, n)) * inv).astype(_BF)
                else:
                    cols = slice(n - TQ, n)
                    tot = acc_v[:, cols] + row_v[1:2, cols] * _dot_nt(wot_v[h], live.pop(t))
                    acc_v[:, cols] = tot
                    o_v[:, cols] = tot.astype(o_v.dtype)
                    stored.add(t)
                    for a, b in zip(cuts[:-1], cuts[1:]):
                        if a <= t < b and stored.issuperset(range(a, b)):
                            pl.when(h == H - 1)(
                                copy(o_v.at[:, a * TQ:b * TQ], out_hbm.at[:, a * TQ:b * TQ], 0).start)

        with scope("loop"):
            lax.fori_loop(0, H, head, None)
        with scope("tail"):
            copy(o_v, out_hbm, 0).wait()

    def fn(A_x, A_c_kv, A_w_q, A_w_uk, A_w_uv, A_w_o, B_x, B_w_r, B_w_gate, B_w_up, B_w_down, gate_w):
        del B_x
        _, S, M = A_x.shape
        Dc = A_c_kv.shape[2]
        H, D = A_w_q.shape[1:]
        F = B_w_gate.shape[1]
        hbm = pl.BlockSpec(memory_space=pltpu.HBM)
        out_t = pl.pallas_call(
            kernel,
            out_shape=jax.ShapeDtypeStruct((M, S), A_x.dtype),
            in_specs=[hbm] * 11,
            out_specs=hbm,
            scratch_shapes=[
                pltpu.VMEM((M, S), _BF),
                pltpu.VMEM((S, M), _BF),
                pltpu.VMEM((H, S, D), _BF),
                pltpu.VMEM((S, Dc), _BF),
                pltpu.VMEM((H // 2, M, D), jnp.uint32),
                pltpu.VMEM((H // 2, Dc, D), jnp.uint32),
                pltpu.VMEM((H // 2, Dc, D), jnp.uint32),
                pltpu.VMEM((4, Dc, D), _BF),
                pltpu.VMEM((H, M, D), _BF),
                pltpu.VMEM((M,), _BF),
                pltpu.VMEM((M,), _BF),
                pltpu.VMEM((M, F), _BF),
                pltpu.VMEM((M, F), _BF),
                pltpu.VMEM((M, F), _BF),
                pltpu.VMEM((M, S), _F32),
                pltpu.VMEM((8, S), _F32),
                pltpu.VMEM((2, M, _LANES), _F32),
                pltpu.VMEM((2, M, _LANES), _F32),
                pltpu.VMEM((2, M, _LANES), _F32),
                pltpu.VMEM((M, S), _BF),
                pltpu.SMEM((2,), jnp.int32),
                pltpu.SemaphoreType.DMA((8,)),
            ],
            compiler_params=pltpu.CompilerParams(vmem_limit_bytes=110 * 2**20, flags=cfg.get("flags")),
            name=cfg.get("name", "gm"),
        )(A_x[0].T, A_c_kv[0], A_w_q, A_w_uk, A_w_uv, A_w_o.transpose(0, 2, 1), B_w_r, B_w_gate, B_w_up,
          B_w_down.T, gate_w)
        return out_t.T[None]

    return fn


_IMPL = make({'SEQ': 'k0 R F k1 K k2 k3 V v0 v1 v2 q15 S v3 q14 q13 p15 q12 p14 q11 p13 q10 p12 p11 q9 o15 q8 p10 o14 q7 p9 o13 q6 p8 o12 p7 q5 o11 q4 p6 o10 q3 o9 q2 o8 p4 p5 q1 p3 o7 q0 p2 o6 p1 o5 p0 o4 o3 o2 o1 o0'})


@jax.jit
def pallas_gated_mix__compressed_kv_cla__moe_arch_mod__prompt_kernel(
    A_x, A_c_kv, A_w_q, A_w_uk, A_w_uv, A_w_o, B_x, B_w_r, B_w_gate, B_w_up, B_w_down, gate_w
):
    return _IMPL(A_x, A_c_kv, A_w_q, A_w_uk, A_w_uv, A_w_o, B_x, B_w_r, B_w_gate, B_w_up, B_w_down, gate_w)
```

```python
import math

import jax
import jax.numpy as jnp
import numpy as np
from jax import lax
from jax.experimental import pallas as pl
from jax.experimental.pallas import tpu as pltpu

_BF16 = jnp.bfloat16
_F32 = jnp.float32
_LOG2E = math.log2(math.e)
_LANES = 128
_BLOCK = 512

_HEAD_STAGES = (
    "k0 R k1 k2 k3 F V K v0 v1 v2 q15 S v3 q14 q13 p15 q12 p14 q11 p13 q10 p12 p11 q9 o15 q8 p10 o14 "
    "q7 p9 o13 q6 p8 o12 p7 q5 o11 q4 p6 o10 q3 o9 q2 o8 p4 p5 q1 p3 o7 q0 p2 o6 p1 o5 p0 o4 o3 o2 o1 o0"
)


def _dot(a, b):
    return jnp.dot(a, b, preferred_element_type=_F32)


def _dot_nt(a, b):
    return lax.dot_general(a, b, (((1,), (1,)), ((), ())), preferred_element_type=_F32)


def _pick_head(words, odd):
    if isinstance(odd, int):
        bits = words & np.uint32(0xFFFF0000) if odd else words << 16
    else:
        bits = (words >> (odd * 16).astype(jnp.uint32)) << 16
    return lax.bitcast_convert_type(bits, _F32).astype(_BF16)


def _column(vec):
    n = vec.shape[0]
    return jnp.broadcast_to(vec.astype(_F32).reshape(1, n), (_LANES, n)).T


def _kernel(
    xt_hbm, c_hbm, wq_hbm, wk_hbm, wv_hbm, wot_hbm, wr_hbm, wg_hbm, wu_hbm, wdt_hbm, gw_hbm,
    out_hbm,
    xt_v,
    x_v,
    q_v,
    c_v,
    wq_v, wk_v, wv_v,
    wb_v,
    wot_v,
    wr_v, gw_v, wg_v, wu_v, wdt_v,
    acc_v,
    row_v,
    col_v,
    xs_v,
    y_v,
    o_v,
    idx_s,
    sems,
):
    M, S = xt_v.shape
    H, _, D = q_v.shape
    n_ffn = wg_v.shape[1] // _LANES
    q_scale = (D ** -0.5) * _LOG2E
    masked = -1e9 * _LOG2E

    def copy(src, dst, sem):
        return pltpu.make_async_copy(src, dst, sems.at[sem])

    def pair_copy(src, dst, p, sem):
        return copy(src.bitcast(jnp.uint32).at[:, p, :], dst.at[p], sem)

    def token_tile(i):
        start = pl.multiple_of((i // _LANES) * _LANES, _LANES)
        hit = lax.broadcasted_iota(jnp.int32, (1, _LANES), 1) == i - start
        return pl.ds(start, _LANES), hit

    def project_q(h, rows):
        w = _pick_head(wq_v[h // 2], h % 2)
        q_v[h, rows, :] = (_dot(x_v[rows, :], w) * q_scale).astype(_BF16)

    def token_stats(cols):
        xb = xt_v[:, cols].astype(_F32)
        r = jnp.sum(xb * col_v[0], axis=0, keepdims=True).astype(_BF16).astype(_F32)
        g = jax.nn.sigmoid(jnp.sum(xb * col_v[1], axis=0, keepdims=True))
        row_v[0:1, cols] = r
        row_v[1:2, cols] = g
        row_v[2:3, cols] = jax.nn.sigmoid(r) * (1.0 - g)
        acc_v[:, cols] = (1.0 - g) * xb

    def route():
        r = row_v[0:1, :]
        lane = lax.broadcasted_iota(jnp.int32, (1, S), 1)
        key = jnp.where(r != r, -jnp.inf, r)
        i1 = jnp.min(jnp.where(key == jnp.max(key), lane, S - 1))
        key = jnp.where(lane == i1, -jnp.inf, key)
        i2 = jnp.min(jnp.where((key == jnp.max(key)) & (lane != i1), lane, S - 1))
        idx_s[0] = i1
        idx_s[1] = i2
        for e, i in enumerate((i1, i2)):
            cols, hit = token_tile(i)
            xe = jnp.sum(jnp.where(hit, xt_v[:, cols].astype(_F32), 0.0), axis=1, keepdims=True)
            xs_v[e] = jnp.broadcast_to(xe, (M, _LANES))

    def ffn_chunk(h):
        cols = pl.ds(pl.multiple_of(jnp.minimum(h, n_ffn - 1) * _LANES, _LANES), _LANES)
        wg = wg_v[:, cols].astype(_F32)
        wu = wu_v[:, cols].astype(_F32)
        wd = wdt_v[:, cols].astype(_F32)
        for e in range(2):
            xe = xs_v[e]
            a = jnp.sum(wg * xe, axis=0, keepdims=True)
            u = jnp.sum(wu * xe, axis=0, keepdims=True)
            y_v[e] += wd * (a * jax.nn.sigmoid(a) * u)

    def ffn_reduce(slot):
        for e in range(2):
            ye = jnp.sum(y_v[e], axis=1, keepdims=True)
            wb_v[slot, :M, e * _LANES:(e + 1) * _LANES] = jnp.broadcast_to(ye, (M, _LANES)).astype(_BF16)

    def ffn_scatter():
        for e in range(2):
            cols, hit = token_tile(idx_s[e])
            ye = wb_v[3 - (n_ffn - 1) % 2, :M, e * _LANES:(e + 1) * _LANES].astype(_F32)
            acc_v[:, cols] += jnp.where(hit, ye * row_v[2:3, cols], 0.0)

    spans = [slice(0, _BLOCK), slice(_BLOCK, 2 * _BLOCK), slice(2 * _BLOCK, S)]
    x_copies = [copy(xt_hbm.at[:, s], xt_v.at[:, s], 1 + n) for n, s in enumerate(spans)]
    groups = [
        [copy(wr_hbm, wr_v, 0), copy(gw_hbm, gw_v, 0)],
        [pair_copy(wq_hbm, wq_v, 0, 1), x_copies[0]],
        [x_copies[1]],
        [x_copies[2]],
        [pair_copy(wq_hbm, wq_v, p, 4) for p in range(1, H // 2)],
        [copy(c_hbm, c_v, 5), pair_copy(wk_hbm, wk_v, 0, 5), pair_copy(wv_hbm, wv_v, 0, 5),
         copy(wot_hbm, wot_v, 5), copy(wg_hbm, wg_v, 5), copy(wu_hbm, wu_v, 5), copy(wdt_hbm, wdt_v, 5)],
        [pair_copy(wk_hbm, wk_v, p, 6) for p in range(1, H // 2)],
        [pair_copy(wv_hbm, wv_v, p, 7) for p in range(1, H // 2)],
    ]

    def wait_group(g):
        for c in groups[g]:
            c.wait()

    for group in groups:
        for c in group:
            c.start()
    y_v[...] = jnp.zeros_like(y_v)
    wait_group(0)
    col_v[0] = _column(wr_v[...])
    col_v[1] = _column(gw_v[...])

    for n, rows in enumerate(spans):
        wait_group(1 + n)
        if n:
            project_q(1, spans[n - 1])
        x_v[rows, :] = xt_v[:, rows].T
        project_q(0, rows)
    project_q(1, spans[-1])
    wait_group(4)

    def q_block(b, _):
        rows = pl.ds(pl.multiple_of(b * _BLOCK, _BLOCK), _BLOCK)
        for h in range(2, H):
            project_q(h, rows)
            t, due = divmod(h - 2, 2)
            if due and t < _BLOCK // _LANES:
                token_stats(pl.ds(pl.multiple_of(b * _BLOCK + t * _LANES, _LANES), _LANES))

    lax.fori_loop(0, S // _BLOCK, q_block, None)
    wait_group(5)
    wb_v[0] = _pick_head(wk_v[0], 0)

    def head(h, _):
        odd = h % 2

        @pl.when(h == 1)
        def _():
            copy(wk_v.at[1:], wk_v.at[1:], 6).wait()
            copy(wv_v.at[1:], wv_v.at[1:], 7).wait()

        pl.when(h == n_ffn)(ffn_scatter)

        causal = (lax.broadcasted_iota(jnp.int32, (_LANES, _LANES), 1)
                  <= lax.broadcasted_iota(jnp.int32, (_LANES, _LANES), 0))
        k, v, live, done = {}, {}, {}, set()

        def first_rows(blocks, n):
            full, rest = divmod(n, _BLOCK)
            parts = [blocks[b] for b in range(full)] + ([blocks[full][:rest]] if rest else [])
            return jnp.concatenate(parts, axis=0)

        for stage in _HEAD_STAGES.split():
            op, t = stage[0], int(stage[1:] or 0)
            n = (t + 1) * _LANES
            if op == "k":
                k[t] = _dot(c_v[t * _BLOCK:(t + 1) * _BLOCK, :], wb_v[odd]).astype(_BF16)
            elif op == "v":
                v[t] = _dot(c_v[t * _BLOCK:(t + 1) * _BLOCK, :], wb_v[2 + odd]).astype(_BF16)
            elif op == "V":
                wb_v[2 + odd] = _pick_head(wv_v[h // 2], odd)
            elif op == "K":
                wb_v[1 - odd] = _pick_head(wk_v[jnp.minimum(h + 1, H - 1) // 2], 1 - odd)
            elif op == "R":
                route()
            elif op == "F":
                ffn_chunk(h)
            elif op == "S":
                ffn_reduce(3 - odd)
            elif op == "q":
                s = _dot_nt(q_v[h, n - _LANES:n, :], first_rows(k, n))
                diag = jnp.where(causal, s[:, n - _LANES:], masked)
                s = jnp.concatenate([s[:, :n - _LANES], diag], axis=1) if t else diag
                p = jnp.exp2(s - jnp.max(s, axis=1, keepdims=True))
                live[t] = p.astype(_BF16), 1.0 / jnp.sum(p, axis=1, keepdims=True)
            elif op == "p":
                p, inv = live[t]
                live[t] = (_dot(p, first_rows(v, n)) * inv).astype(_BF16)
            else:
                cols = slice(n - _LANES, n)
                total = acc_v[:, cols] + row_v[1:2, cols] * _dot_nt(wot_v[h], live.pop(t))
                acc_v[:, cols] = total
                o_v[:, cols] = total.astype(o_v.dtype)
                done.add(t)
                if t ^ 1 in done:
                    cols = slice(t // 2 * 2 * _LANES, (t // 2 + 1) * 2 * _LANES)
                    pl.when(h == H - 1)(copy(o_v.at[:, cols], out_hbm.at[:, cols], 0).start)

    lax.fori_loop(0, H, head, None)
    copy(o_v, out_hbm, 0).wait()


@jax.jit
def pallas_gated_mix__compressed_kv_cla__moe_arch_mod__prompt_kernel(
    A_x: jax.Array,
    A_c_kv: jax.Array,
    A_w_q: jax.Array,
    A_w_uk: jax.Array,
    A_w_uv: jax.Array,
    A_w_o: jax.Array,
    B_x: jax.Array,
    B_w_r: jax.Array,
    B_w_gate: jax.Array,
    B_w_up: jax.Array,
    B_w_down: jax.Array,
    gate_w: jax.Array,
):
    del B_x
    B, S, M = A_x.shape
    Dc = A_c_kv.shape[2]
    H, D = A_w_q.shape[1:]
    F = B_w_gate.shape[1]
    assert B == 1 and S == A_c_kv.shape[1] == 16 * _LANES
    assert H % 2 == 0 and H >= 10 and D == 2 * _LANES and M <= Dc
    assert F % _LANES == 0 and F // _LANES < H

    hbm = pl.BlockSpec(memory_space=pltpu.HBM)
    out_t = pl.pallas_call(
        _kernel,
        out_shape=jax.ShapeDtypeStruct((M, S), A_x.dtype),
        in_specs=[hbm] * 11,
        out_specs=hbm,
        scratch_shapes=[
            pltpu.VMEM((M, S), _BF16),
            pltpu.VMEM((S, M), _BF16),
            pltpu.VMEM((H, S, D), _BF16),
            pltpu.VMEM((S, Dc), _BF16),
            pltpu.VMEM((H // 2, M, D), jnp.uint32),
            pltpu.VMEM((H // 2, Dc, D), jnp.uint32),
            pltpu.VMEM((H // 2, Dc, D), jnp.uint32),
            pltpu.VMEM((4, Dc, D), _BF16),
            pltpu.VMEM((H, M, D), _BF16),
            pltpu.VMEM((M,), _BF16),
            pltpu.VMEM((M,), _BF16),
            pltpu.VMEM((M, F), _BF16),
            pltpu.VMEM((M, F), _BF16),
            pltpu.VMEM((M, F), _BF16),
            pltpu.VMEM((M, S), _F32),
            pltpu.VMEM((8, S), _F32),
            pltpu.VMEM((2, M, _LANES), _F32),
            pltpu.VMEM((2, M, _LANES), _F32),
            pltpu.VMEM((2, M, _LANES), _F32),
            pltpu.VMEM((M, S), A_x.dtype),
            pltpu.SMEM((2,), jnp.int32),
            pltpu.SemaphoreType.DMA((8,)),
        ],
        compiler_params=pltpu.CompilerParams(vmem_limit_bytes=110 * 2**20),
        name="gated_mix",
    )(A_x[0].T, A_c_kv[0], A_w_q, A_w_uk, A_w_uv, A_w_o.transpose(0, 2, 1), B_w_r, B_w_gate, B_w_up,
      B_w_down.T, gate_w)
    return out_t.T[None]
```
